```python
import jax
import jax.numpy as jnp

def _softmax(x, axis=-1):
    return jax.nn.softmax(x, axis=axis)

def _gelu(x):
    return jax.nn.gelu(x, approximate=True)

def _silu(x):
    return jax.nn.silu(x)

def _sigmoid(x):
    return jax.nn.sigmoid(x)

def _layernorm(x, axis=-1, eps=1e-05):
    m = jnp.mean(x, axis=axis, keepdims=True)
    v = jnp.var(x, axis=axis, keepdims=True)
    return (x - m) / jnp.sqrt(v + eps)

def _scatter_add(tgt, idx, src, axis=0):
    return tgt.at[idx].add(src)

def _segment_sum(src, seg, n):
    return jax.ops.segment_sum(src, seg, n)

class _Rng:

    def __init__(self, key):
        self._k = key

    def _next(self):
        self._k, sub = jax.random.split(self._k)
        return sub

    def normal(self, shape):
        return jax.random.normal(self._next(), shape, dtype=jnp.bfloat16)

    def randint(self, lo, hi, shape):
        return jax.random.randint(self._next(), shape, lo, hi, dtype=jnp.int32)

    def uniform(self, shape, lo=0.0, hi=1.0):
        return jax.random.uniform(self._next(), shape, jnp.bfloat16, lo, hi)

    def permutation(self, n):
        return jax.random.permutation(self._next(), n)
kernel_name = 'interleave_layers__linear_kernel_hedgehog__mixer_gmlp__prompt'

def _fwd_setup_inputs():
    _rng = _Rng(jax.random.key(int.from_bytes(__import__("os").urandom(4), "little")))
    _w = lambda a: (lambda t: t.astype(jnp.bfloat16) if jnp.issubdtype(t.dtype, jnp.floating) else t)(jnp.asarray(a))

    def _A_setup():
        B, S, D, H = (1, 2048, 640, 32)
        Dh = D // H
        return {'x': _w((lambda *s: _rng.normal(s) * 0.05)(B, S, D)), 'wqkv': _w((lambda *s: _rng.normal(s) * 0.05)(D, 3 * D)), 'w_phi': _w((lambda *s: _rng.normal(s) * 0.05)(H, Dh, Dh) * Dh ** (-0.5)), 'wo': _w((lambda *s: _rng.normal(s) * 0.05)(D, D))}
    _A_in = _A_setup()

    def _B_setup():
        B, S, D, F = (1, 2048, 640, 1536)
        Fh = F // 2
        return {'x': _w((lambda *s: _rng.normal(s) * 0.05)(B, S, D)), 'w_in': _w((lambda *s: _rng.normal(s) * 0.05)(D, 2 * Fh)), 'w_sp': _w(0.01 * (lambda *s: _rng.normal(s) * 0.05)(S, S)), 'b_sp': _w(1.0 + 0.01 * (lambda *s: _rng.normal(s) * 0.05)(S)), 'w_out': _w((lambda *s: _rng.normal(s) * 0.05)(Fh, D))}
    _B_in = _B_setup()
    return {'A_x': _A_in['x'], 'A_wqkv': _A_in['wqkv'], 'A_w_phi': _A_in['w_phi'], 'A_wo': _A_in['wo'], 'B_x': _B_in['x'], 'B_w_in': _B_in['w_in'], 'B_w_sp': _B_in['w_sp'], 'B_b_sp': _B_in['b_sp'], 'B_w_out': _B_in['w_out']}

def _fwd_reference(A_x, A_wqkv, A_w_phi, A_wo, B_x, B_w_in, B_w_sp, B_b_sp, B_w_out):

    def _A_ref(x, wqkv, w_phi, wo):
        B, S, D = x.shape
        H = 32
        Dh = D // H
        qkv = (lambda x, *d: x.transpose(*d))((x @ wqkv).reshape(B, S, 3, H, Dh), 2, 0, 3, 1, 4)
        q, k, v = (qkv[0], qkv[1], qkv[2])
        pq = jnp.einsum('bhsd,hdf->bhsf', q, w_phi)
        pk = jnp.einsum('bhsd,hdf->bhsf', k, w_phi)
        phi_q = jnp.concatenate([_softmax(pq, axis=-1), _softmax(-pq, axis=-1)], axis=-1)
        phi_k = jnp.concatenate([_softmax(pk, axis=-1), _softmax(-pk, axis=-1)], axis=-1)
        kv = jnp.einsum('bhsf,bhsd->bhfd', phi_k, v)
        z = jnp.einsum('bhsf->bhf', phi_k)
        num = jnp.einsum('bhqf,bhfd->bhqd', phi_q, kv)
        den = jnp.einsum('bhqf,bhf->bhq', phi_q, z)[..., None] + 1e-06
        o = num / den
        return (lambda x, *d: x.transpose(*d))(o, 0, 2, 1, 3).reshape(B, S, D) @ wo

    def _B_ref(x, w_in, w_sp, b_sp, w_out):
        B, S, D = x.shape
        F = w_in.shape[-1]
        Fh = F // 2
        z = _gelu(jnp.einsum('bsd,df->bsf', x, w_in))
        z1 = z[..., :Fh].copy()
        z2 = _layernorm(z[..., Fh:], axis=-1)
        g = jnp.einsum('ts,bsf->btf', w_sp, z2) + b_sp[None, :, None]
        return jnp.einsum('bsf,fd->bsd', z1 * g, w_out)
    x = A_x
    x = x + _A_ref(_layernorm(x, axis=-1), A_wqkv, A_w_phi, A_wo)
    x = x + _B_ref(_layernorm(x, axis=-1), B_w_in, B_w_sp, B_b_sp, B_w_out)
    x = x + _A_ref(_layernorm(x, axis=-1), A_wqkv, A_w_phi, A_wo)
    x = x + _B_ref(_layernorm(x, axis=-1), B_w_in, B_w_sp, B_b_sp, B_w_out)
    return x

def setup_inputs():
    _inp = _fwd_setup_inputs()
    _gk = jax.random.fold_in(jax.random.key(int.from_bytes(__import__("os").urandom(4), "little")), 2 ** 31 - 1)
    _shapes = [[1, 2048, 640]]
    _dtypes = ['bfloat16']
    _gks = jax.random.split(_gk, len(_shapes))
    _gs = [jax.random.normal(k, s, dtype=jnp.dtype(d)) * 0.05 for k, s, d in zip(_gks, _shapes, _dtypes)]
    _inp['grad_out'] = _gs[0]
    return _inp

def reference(A_x, A_wqkv, A_w_phi, A_wo, B_w_in, B_w_sp, B_b_sp, B_w_out, B_x, grad_out):
    _const = dict(B_x=B_x)

    def _f(*_d):
        return _fwd_reference(**{'A_x': _d[0], 'A_wqkv': _d[1], 'A_w_phi': _d[2], 'A_wo': _d[3], 'B_w_in': _d[4], 'B_w_sp': _d[5], 'B_b_sp': _d[6], 'B_w_out': _d[7], **_const})
    _out, _vjp = jax.vjp(_f, A_x, A_wqkv, A_w_phi, A_wo, B_w_in, B_w_sp, B_b_sp, B_w_out)
    _grads = _vjp(grad_out)
    _out0 = jnp.asarray(_out)
    return (_out0, *[jnp.asarray(_g) for _g in _grads])
```

```python
import functools

import jax
import jax.numpy as jnp
import jax.experimental.pallas as pl
import jax.experimental.pallas.tpu as pltpu

F32 = jnp.float32
BF16 = jnp.bfloat16

S = 2048
D = 640
H = 32
DH = 20
F2 = 2 * DH * H
FF = 1536
FH = 768
EPS = 1e-5
R = 256
NCH = S // R
NSL = D // 128

_C0 = 0.7978845608028654
_C1 = 0.044715


def _nn(a, b):
    return jnp.dot(a, b, preferred_element_type=F32)


def _nt(a, b):
    return jax.lax.dot_general(a, b, (((1,), (1,)), ((), ())), preferred_element_type=F32)


def _tn(a, b):
    return jax.lax.dot_general(a, b, (((0,), (0,)), ((), ())), preferred_element_type=F32)


def _ln(x):
    m = jnp.mean(x, axis=-1, keepdims=True)
    xc = x - m
    v = jnp.mean(xc * xc, axis=-1, keepdims=True)
    rstd = jax.lax.rsqrt(v + EPS)
    return xc * rstd, rstd


def _ln_bwd(dxn, xn, rstd):
    a = jnp.mean(dxn, axis=-1, keepdims=True)
    b = jnp.mean(dxn * xn, axis=-1, keepdims=True)
    return rstd * (dxn - a - xn * b)


def _gelu(x):
    t = jnp.tanh(_C0 * (x + _C1 * x * x * x))
    return 0.5 * x * (1.0 + t), t


def _gelu_grad(x, t):
    return 0.5 * (1.0 + t) + 0.5 * x * (1.0 - t * t) * _C0 * (1.0 + 3.0 * _C1 * x * x)


def _grp(a, op):
    a = op(a, pltpu.roll(a, 64, 1))
    a = op(a, pltpu.roll(a, 32, 1))
    return a


def _slabs(a, n):
    return [a[:, j * 128:(j + 1) * 128] for j in range(n)]


def _sum_list(xs):
    acc = xs[0]
    for t in xs[1:]:
        acc = acc + t
    return acc


def _feat(p):
    sl = _slabs(p, NSL)
    mx = sl[0]
    mn = sl[0]
    for t in sl[1:]:
        mx = jnp.maximum(mx, t)
        mn = jnp.minimum(mn, t)
    mx = _grp(mx, jnp.maximum)
    mn = _grp(mn, jnp.minimum)
    ep = [jnp.exp(t - mx) for t in sl]
    en = [jnp.exp(mn - t) for t in sl]
    ip = 1.0 / _grp(_sum_list(ep), jnp.add)
    inn = 1.0 / _grp(_sum_list(en), jnp.add)
    return [e * ip for e in ep] + [e * inn for e in en]


def _feat_bwd(phi, dphi):
    t = [a * b for a, b in zip(phi, dphi)]
    sp = _grp(_sum_list(t[:NSL]), jnp.add)
    sn = _grp(_sum_list(t[NSL:]), jnp.add)
    return [(t[j] - phi[j] * sp) - (t[j + NSL] - phi[j + NSL] * sn) for j in range(NSL)]


def _cat(xs):
    return jnp.concatenate(xs, axis=1)


def _rows(i):
    return pl.ds(pl.multiple_of(i * R, R), R)


def _kernel(
    x_hbm, wqkv_hbm, wphi_hbm, wo_hbm, win_hbm, wsp_hbm, bsp_hbm, wout_hbm, gout_hbm,
    out_hbm, gx_hbm, gwqkv_hbm, gwphi_hbm, gwo_hbm, gwin_hbm, gwsp_hbm, gbsp_hbm, gwout_hbm,
    x_s, xin_s, out_s, wqkv_s, wphi_s, wo_s, wop_s, win_s, wsp_s, bsp_s, gb_s, gbo_s, wout_s,
    wbig_s, xn_s, rstd_s, p_s, o_s, kvt_s, z_s, kvacc, zacc, dkvt_s, h_s, z2n_s, g_s,
    dwbig, dwo, dwin, dwout, gwphi_s, sems,
):
    def cp(src, dst, k):
        return pltpu.make_async_copy(src, dst, sems.at[k])

    c_x = cp(x_hbm, xin_s, 0)
    c_wqkv = cp(wqkv_hbm, wqkv_s, 1)
    c_wphi = cp(wphi_hbm, wphi_s, 2)
    c_wo = cp(wo_hbm, wo_s, 3)
    c_win = cp(win_hbm, win_s, 4)
    c_wsp = cp(wsp_hbm, wsp_s, 5)
    c_bsp = cp(bsp_hbm, bsp_s, 6)
    c_wout = cp(wout_hbm, wout_s, 7)
    for c in (c_x, c_wqkv, c_wphi, c_wo, c_win, c_wsp, c_bsp, c_wout):
        c.start()

    def iota(shape, dim):
        return jax.lax.broadcasted_iota(jnp.int32, shape, dim)

    def perm_mat():
        r = iota((D, D), 0)
        c = iota((D, D), 1)
        return jnp.where(r == DH * (c & 31) + (c >> 5), 1.0, 0.0).astype(BF16)

    def perm_mat_t():
        r = iota((D, D), 0)
        c = iota((D, D), 1)
        return jnp.where(c == DH * (r & 31) + (r >> 5), 1.0, 0.0).astype(BF16)

    def expand_mat():
        r = iota((128, D), 0)
        c = iota((128, D), 1)
        return jnp.where(r == (c >> 5), 1.0, 0.0).astype(BF16)

    def head_mask():
        r = iota((D, D), 0)
        c = iota((D, D), 1)
        lo = DH * (c & 31)
        return jnp.logical_and(r >= lo, r < lo + DH)

    def wphi_big():
        rep = _nn(wphi_s[...], expand_mat())
        return jnp.where(head_mask(), rep, 0.0).astype(BF16)

    def kv_mask():
        r = iota((D, F2), 0)
        c = iota((D, F2), 1)
        return (r & 31) == (c & 31)

    c_wqkv.wait()
    c_wphi.wait()
    c_wo.wait()
    wpb = wphi_big()
    wbig_s[:, 0:D] = _nn(wqkv_s[:, 0:D], wpb).astype(BF16)
    wbig_s[:, D:2 * D] = _nn(wqkv_s[:, D:2 * D], wpb).astype(BF16)
    wbig_s[:, 2 * D:3 * D] = _nn(wqkv_s[:, 2 * D:3 * D], perm_mat()).astype(BF16)
    wop_s[...] = _nn(perm_mat_t(), wo_s[...]).astype(BF16)

    c_x.wait()
    x_s[...] = xin_s[...].astype(F32)
    c_gout = cp(gout_hbm, xin_s, 8)
    c_gout.start()

    dwbig[...] = jnp.zeros_like(dwbig)
    dwo[...] = jnp.zeros_like(dwo)
    dwin[...] = jnp.zeros_like(dwin)
    dwout[...] = jnp.zeros_like(dwout)
    gb_s[...] = jnp.zeros_like(gb_s)

    def pre_ln(layer, r):
        xn, rstd = _ln(x_s[r, :])
        xnb = xn.astype(BF16)
        xn_s[layer, r, :] = xnb
        rstd_s[r, layer:layer + 1] = rstd
        return xnb

    def a_fwd(layer):
        a = layer // 2
        kvacc[...] = jnp.zeros_like(kvacc)
        zacc[...] = jnp.zeros_like(zacc)

        def loop1(i, carry):
            r = _rows(i)
            xnb = pre_ln(layer, r)
            pb = _nn(xnb, wbig_s[...]).astype(BF16)
            p_s[a, r, :] = pb
            phik = _cat(_feat(pb[:, D:2 * D].astype(F32)))
            kvacc[...] += _tn(pb[:, 2 * D:3 * D], phik.astype(BF16))
            zacc[...] += jnp.sum(phik, axis=0, keepdims=True)
            return carry

        jax.lax.fori_loop(0, NCH, loop1, 0)
        kvt_s[a] = jnp.where(kv_mask(), kvacc[...], 0.0).astype(BF16)
        z_s[a] = zacc[...]

        def loop2(i, carry):
            r = _rows(i)
            phiq = _feat(p_s[a, r, 0:D].astype(F32))
            z = _slabs(z_s[a], 10)
            num = _nt(_cat(phiq).astype(BF16), kvt_s[a])
            den = _grp(_sum_list([pq * zz for pq, zz in zip(phiq, z)]), jnp.add) + 1e-6
            inv = 1.0 / den
            ob = _cat([t * inv for t in _slabs(num, NSL)]).astype(BF16)
            o_s[a, r, :] = ob
            x_s[r, :] += _nn(ob, wop_s[...])
            return carry

        jax.lax.fori_loop(0, NCH, loop2, 0)

    def b_fwd(layer):
        b = layer // 2

        def loop1(i, carry):
            r = _rows(i)
            xnb = pre_ln(layer, r)
            hb = _nn(xnb, win_s[...]).astype(BF16)
            h_s[b, r, :] = hb
            z2, _ = _gelu(hb[:, FH:].astype(F32))
            z2n, _ = _ln(z2)
            z2n_s[b, r, :] = z2n.astype(BF16)
            return carry

        jax.lax.fori_loop(0, NCH, loop1, 0)

        def loop2(i, carry):
            r = _rows(i)
            g = _nn(wsp_s[r, :], z2n_s[b]) + bsp_s[r, :].astype(F32)
            gb = g.astype(BF16)
            g_s[b, r, :] = gb
            z1, _ = _gelu(h_s[b, r, 0:FH].astype(F32))
            u = (z1 * gb.astype(F32)).astype(BF16)
            x_s[r, :] += _nn(u, wout_s[...])
            return carry

        jax.lax.fori_loop(0, NCH, loop2, 0)

    a_fwd(0)
    c_win.wait()
    c_wsp.wait()
    c_bsp.wait()
    c_wout.wait()
    b_fwd(1)
    a_fwd(2)
    b_fwd(3)

    out_s[...] = x_s[...].astype(BF16)
    c_out = cp(out_s, out_hbm, 9)
    c_out.start()

    c_gout.wait()
    x_s[...] = xin_s[...].astype(F32)

    def b_bwd(layer):
        b = layer // 2

        def loop1(i, carry):
            r = _rows(i)
            dyb = x_s[r, :].astype(BF16)
            du = _nt(dyb, wout_s[...])
            h1 = h_s[b, r, 0:FH].astype(F32)
            z1, t1 = _gelu(h1)
            g = g_s[b, r, :].astype(F32)
            u = (z1 * g).astype(BF16)
            dwout[...] += _tn(u, dyb)
            dg = du * z1
            g_s[b, r, :] = dg.astype(BF16)
            gb_s[r, :] += jnp.sum(dg, axis=-1, keepdims=True)
            h_s[b, r, 0:FH] = (du * g * _gelu_grad(h1, t1)).astype(BF16)
            return carry

        jax.lax.fori_loop(0, NCH, loop1, 0)

        def loop2(i, carry):
            r = _rows(i)
            dz2n = _tn(wsp_s[:, r], g_s[b])
            h2 = h_s[b, r, FH:].astype(F32)
            z2, t2 = _gelu(h2)
            z2n, rstd2 = _ln(z2)
            dz2 = _ln_bwd(dz2n, z2n, rstd2)
            h_s[b, r, FH:] = (dz2 * _gelu_grad(h2, t2)).astype(BF16)
            dh = h_s[b, r, :]
            dxn = _nt(dh, win_s[...])
            xnb = xn_s[layer, r, :]
            dwin[...] += _tn(xnb, dh)
            x_s[r, :] += _ln_bwd(dxn, xnb.astype(F32), rstd_s[r, layer:layer + 1])
            return carry

        jax.lax.fori_loop(0, NCH, loop2, 0)

    def a_bwd(layer):
        a = layer // 2
        kvacc[...] = jnp.zeros_like(kvacc)
        zacc[...] = jnp.zeros_like(zacc)

        def loop1(i, carry):
            r = _rows(i)
            dyb = x_s[r, :].astype(BF16)
            do = _slabs(_nt(dyb, wop_s[...]), NSL)
            ob = o_s[a, r, :]
            dwo[...] += _tn(ob, dyb)
            o = _slabs(ob.astype(F32), NSL)
            phiq = _feat(p_s[a, r, 0:D].astype(F32))
            z = _slabs(z_s[a], 10)
            den = _grp(_sum_list([pq * zz for pq, zz in zip(phiq, z)]), jnp.add) + 1e-6
            inv = 1.0 / den
            dnum = _cat([t * inv for t in do]).astype(BF16)
            dden = -_grp(_sum_list([u * w for u, w in zip(do, o)]), jnp.add) * inv
            dphiq = _slabs(_nn(dnum, kvt_s[a]), 10)
            dphiq = [t + dden * zz for t, zz in zip(dphiq, z)]
            kvacc[...] += _tn(dnum, _cat(phiq).astype(BF16))
            zacc[...] += jnp.sum(_cat([pq * dden for pq in phiq]), axis=0, keepdims=True)
            p_s[a, r, 0:D] = _cat(_feat_bwd(phiq, dphiq)).astype(BF16)
            return carry

        jax.lax.fori_loop(0, NCH, loop1, 0)
        dkvt_s[...] = jnp.where(kv_mask(), kvacc[...], 0.0).astype(BF16)

        def loop2(i, carry):
            r = _rows(i)
            phik = _feat(p_s[a, r, D:2 * D].astype(F32))
            vb = p_s[a, r, 2 * D:3 * D]
            dphik = _slabs(_nn(vb, dkvt_s[...]) + zacc[...], 10)
            dv = _nt(_cat(phik).astype(BF16), dkvt_s[...])
            p_s[a, r, D:2 * D] = _cat(_feat_bwd(phik, dphik)).astype(BF16)
            p_s[a, r, 2 * D:3 * D] = dv.astype(BF16)
            dp = p_s[a, r, :]
            dxn = _nt(dp, wbig_s[...])
            xnb = xn_s[layer, r, :]
            dwbig[...] += _tn(xnb, dp)
            x_s[r, :] += _ln_bwd(dxn, xnb.astype(F32), rstd_s[r, layer:layer + 1])
            return carry

        jax.lax.fori_loop(0, NCH, loop2, 0)

    b_bwd(3)
    a_bwd(2)
    b_bwd(1)

    def wsp_loop(i, carry):
        r = _rows(i)
        wsp_s[r, :] = (_nt(g_s[0, r, :], z2n_s[0]) + _nt(g_s[1, r, :], z2n_s[1])).astype(BF16)
        return carry

    jax.lax.fori_loop(0, NCH, wsp_loop, 0)
    win_s[...] = dwin[...].astype(BF16)
    wout_s[...] = dwout[...].astype(BF16)
    gbo_s[...] = gb_s[...].astype(BF16)
    c_gwsp = cp(wsp_s, gwsp_hbm, 10)
    c_gwin = cp(win_s, gwin_hbm, 11)
    c_gwout = cp(wout_s, gwout_hbm, 12)
    c_gb = cp(gbo_s, gbsp_hbm, 13)
    for c in (c_gwsp, c_gwin, c_gwout, c_gb):
        c.start()

    a_bwd(0)

    xin_s[...] = x_s[...].astype(BF16)
    c_gx = cp(xin_s, gx_hbm, 14)
    c_gx.start()

    dq = dwbig[:, 0:D].astype(BF16)
    dk = dwbig[:, D:2 * D].astype(BF16)
    dvv = dwbig[:, 2 * D:3 * D].astype(BF16)
    wpb = wphi_big()
    m = _tn(wqkv_s[:, 0:D], dq) + _tn(wqkv_s[:, D:2 * D], dk)
    m = jnp.where(head_mask(), m, 0.0).astype(BF16)
    gwphi_s[...] = _nt(m, expand_mat()).astype(BF16)
    c_gwphi = cp(gwphi_s, gwphi_hbm, 15)
    c_gwphi.start()
    wbig_s[:, 0:D] = _nt(dq, wpb).astype(BF16)
    wbig_s[:, D:2 * D] = _nt(dk, wpb).astype(BF16)
    wbig_s[:, 2 * D:3 * D] = _nt(dvv, perm_mat()).astype(BF16)
    c_gwqkv = cp(wbig_s, gwqkv_hbm, 16)
    c_gwqkv.start()
    wo_s[...] = _nn(perm_mat(), dwo[...].astype(BF16)).astype(BF16)
    c_gwo = cp(wo_s, gwo_hbm, 17)
    c_gwo.start()

    for c in (c_out, c_gwsp, c_gwin, c_gwout, c_gb, c_gx, c_gwphi, c_gwqkv, c_gwo):
        c.wait()


@jax.jit
def pallas_interleave_layers__linear_kernel_hedgehog__mixer_gmlp__prompt_kernel(
    A_x: jax.Array,
    A_wqkv: jax.Array,
    A_w_phi: jax.Array,
    A_wo: jax.Array,
    B_x: jax.Array,
    B_w_in: jax.Array,
    B_w_sp: jax.Array,
    B_b_sp: jax.Array,
    B_w_out: jax.Array,
    grad_out: jax.Array,
):
    del B_x
    x = A_x.reshape(S, D)
    gout = grad_out.reshape(S, D)
    wphi = jnp.pad(A_w_phi.reshape(D, DH), ((0, 0), (0, 128 - DH)))
    bsp = B_b_sp.reshape(S, 1)

    any_spec = pl.BlockSpec(memory_space=pl.ANY)
    out_shape = (
        jax.ShapeDtypeStruct((S, D), BF16),
        jax.ShapeDtypeStruct((S, D), BF16),
        jax.ShapeDtypeStruct((D, 3 * D), BF16),
        jax.ShapeDtypeStruct((D, 128), BF16),
        jax.ShapeDtypeStruct((D, D), BF16),
        jax.ShapeDtypeStruct((D, FF), BF16),
        jax.ShapeDtypeStruct((S, S), BF16),
        jax.ShapeDtypeStruct((S, 1), BF16),
        jax.ShapeDtypeStruct((FH, D), BF16),
    )
    scratch = [
        pltpu.VMEM((S, D), F32),
        pltpu.VMEM((S, D), BF16),
        pltpu.VMEM((S, D), BF16),
        pltpu.VMEM((D, 3 * D), BF16),
        pltpu.VMEM((D, 128), BF16),
        pltpu.VMEM((D, D), BF16),
        pltpu.VMEM((D, D), BF16),
        pltpu.VMEM((D, FF), BF16),
        pltpu.VMEM((S, S), BF16),
        pltpu.VMEM((S, 1), BF16),
        pltpu.VMEM((S, 1), F32),
        pltpu.VMEM((S, 1), BF16),
        pltpu.VMEM((FH, D), BF16),
        pltpu.VMEM((D, 3 * D), BF16),
        pltpu.VMEM((4, S, D), BF16),
        pltpu.VMEM((S, 128), F32),
        pltpu.VMEM((2, S, 3 * D), BF16),
        pltpu.VMEM((2, S, D), BF16),
        pltpu.VMEM((2, D, F2), BF16),
        pltpu.VMEM((2, 1, F2), F32),
        pltpu.VMEM((D, F2), F32),
        pltpu.VMEM((1, F2), F32),
        pltpu.VMEM((D, F2), BF16),
        pltpu.VMEM((2, S, FF), BF16),
        pltpu.VMEM((2, S, FH), BF16),
        pltpu.VMEM((2, S, FH), BF16),
        pltpu.VMEM((D, 3 * D), F32),
        pltpu.VMEM((D, D), F32),
        pltpu.VMEM((D, FF), F32),
        pltpu.VMEM((FH, D), F32),
        pltpu.VMEM((D, 128), BF16),
        pltpu.SemaphoreType.DMA((18,)),
    ]
    outs = pl.pallas_call(
        _kernel,
        out_shape=out_shape,
        in_specs=[any_spec] * 9,
        out_specs=tuple([any_spec] * 9),
        scratch_shapes=scratch,
        compiler_params=pltpu.CompilerParams(vmem_limit_bytes=127 * 1024 * 1024),
    )(x, A_wqkv, wphi, A_wo, B_w_in, B_w_sp, bsp, B_w_out, gout)
    out, gx, gwqkv, gwphi, gwo, gwin, gwsp, gbsp, gwout = outs
    return (
        out.reshape(1, S, D),
        gx.reshape(1, S, D),
        gwqkv,
        gwphi[:, :DH].reshape(H, DH, DH),
        gwo,
        gwin,
        gwsp,
        gbsp.reshape(S),
        gwout,
    )
```

```python
import functools

import jax
import jax.numpy as jnp
import jax.experimental.pallas as pl
import jax.experimental.pallas.tpu as pltpu

F32 = jnp.float32
BF16 = jnp.bfloat16

S = 2048
D = 640
H = 32
DH = 20
F2 = 2 * DH * H
FF = 1536
FH = 768
EPS = 1e-5
R = 256
NCH = S // R
RR = {}

_C0 = 0.7978845608028654
_C1 = 0.044715


def _nn(a, b):
    return jnp.dot(a, b, preferred_element_type=F32)


def _nt(a, b):
    return jax.lax.dot_general(a, b, (((1,), (1,)), ((), ())), preferred_element_type=F32)


def _tn(a, b):
    return jax.lax.dot_general(a, b, (((0,), (0,)), ((), ())), preferred_element_type=F32)


def _ln(x):
    m = jnp.mean(x, axis=-1, keepdims=True)
    xc = x - m
    v = jnp.mean(xc * xc, axis=-1, keepdims=True)
    rstd = jax.lax.rsqrt(v + EPS)
    return xc * rstd, rstd


def _ln_bwd(dxn, xn, rstd):
    a = jnp.mean(dxn, axis=-1, keepdims=True)
    b = jnp.mean(dxn * xn, axis=-1, keepdims=True)
    return rstd * (dxn - a - xn * b)


def _gelu(x):
    t = jnp.tanh(_C0 * (x + _C1 * x * x * x))
    return 0.5 * x * (1.0 + t), t


def _gelu_grad(x, t):
    return 0.5 * (1.0 + t) + 0.5 * x * (1.0 - t * t) * _C0 * (1.0 + 3.0 * _C1 * x * x)


def _grp(a, op):
    a = op(a, pltpu.roll(a, 64, 1))
    a = op(a, pltpu.roll(a, 32, 1))
    a = op(a, pltpu.roll(a, 16, 1))
    return a


def _slabs(a, n):
    return [a[:, j * 128:(j + 1) * 128] for j in range(n)]


def _cat(xs):
    return jnp.concatenate(xs, axis=1)


def _lo(shape):
    return jax.lax.broadcasted_iota(jnp.int32, shape, 1) < 64


def _head_reduce(t, lo, op, fill):
    a0 = op(op(t[0], t[1]), jnp.where(lo, t[2], fill))
    a1 = op(op(t[3], t[4]), jnp.where(lo, fill, t[2]))
    return _grp(a0, op), _grp(a1, op)


def _head_bcast(r0, r1, lo):
    rx = jnp.where(lo, r0, r1)
    return [r0, r0, rx, r1, r1]


def _feat(p):
    t = _slabs(p, 5)
    lo = _lo(t[0].shape)
    mx = _head_bcast(*_head_reduce(t, lo, jnp.maximum, -jnp.inf), lo)
    mn = _head_bcast(*_head_reduce(t, lo, jnp.minimum, jnp.inf), lo)
    ep = [jnp.exp(a - m) for a, m in zip(t, mx)]
    en = [jnp.exp(m - a) for a, m in zip(t, mn)]
    sp0, sp1 = _head_reduce(ep, lo, jnp.add, 0.0)
    sn0, sn1 = _head_reduce(en, lo, jnp.add, 0.0)
    ip = _head_bcast(1.0 / sp0, 1.0 / sp1, lo)
    inn = _head_bcast(1.0 / sn0, 1.0 / sn1, lo)
    fp = [e * i for e, i in zip(ep, ip)]
    fn = [e * i for e, i in zip(en, inn)]
    fnx = pltpu.roll(fn[2], 64, 1)
    px0 = jnp.where(lo, fp[2], fnx)
    px1 = jnp.where(lo, fnx, fp[2])
    return [fp[0], fp[1], fn[0], fn[1], px0, px1, fp[3], fp[4], fn[3], fn[4]]


def _phi_head_sum(t):
    s0 = (t[0] + t[1]) + (t[2] + t[3]) + t[4]
    s1 = (t[6] + t[7]) + (t[8] + t[9]) + t[5]
    return _grp(s0, jnp.add), _grp(s1, jnp.add)


def _feat_bwd(phi, dphi):
    lo = _lo(phi[0].shape)
    t = [a * b for a, b in zip(phi, dphi)]
    sp0 = _grp(t[0] + t[1] + jnp.where(lo, t[4], 0.0), jnp.add)
    sn0 = _grp(t[2] + t[3] + jnp.where(lo, 0.0, t[4]), jnp.add)
    sp1 = _grp(t[6] + t[7] + jnp.where(lo, 0.0, t[5]), jnp.add)
    sn1 = _grp(t[8] + t[9] + jnp.where(lo, t[5], 0.0), jnp.add)
    d0 = (t[0] - phi[0] * sp0) - (t[2] - phi[2] * sn0)
    d1 = (t[1] - phi[1] * sp0) - (t[3] - phi[3] * sn0)
    d3 = (t[6] - phi[6] * sp1) - (t[8] - phi[8] * sn1)
    d4 = (t[7] - phi[7] * sp1) - (t[9] - phi[9] * sn1)
    a0 = t[4] - phi[4] * jnp.where(lo, sp0, sn0)
    a1 = t[5] - phi[5] * jnp.where(lo, sn1, sp1)
    dx = jnp.where(lo, a0, a1) - pltpu.roll(jnp.where(lo, a1, a0), 64, 1)
    return [d0, d1, dx, d3, d4]


def _bd_nn(a, w):
    return _cat([_nn(a[:, 0:384], w[0:384, 0:256]), _nn(a, w[:, 256:384]), _nn(a[:, 256:D], w[256:D, 384:D])])


def _bd_nt(a, w):
    return _cat([_nt(a[:, 0:384], w[0:256, 0:384]), _nt(a, w[256:384, :]), _nt(a[:, 256:D], w[384:D, 256:D])])


def _bd_left(w, b):
    return jnp.concatenate(
        [_nn(w[0:256, 0:384], b[0:384]), _nn(w[256:384, :], b), _nn(w[384:D, 256:D], b[256:D])], axis=0)


def _rows(i, rr):
    return pl.ds(pl.multiple_of(i * rr, rr), rr)


def _kernel(
    x_hbm, wqkv_hbm, wphi_hbm, wo_hbm, win_hbm, wsp_hbm, bsp_hbm, wout_hbm, gout_hbm,
    out_hbm, gx_hbm, gwqkv_hbm, gwphi_hbm, gwo_hbm, gwin_hbm, gwsp_hbm, gbsp_hbm, gwout_hbm,
    x_s, xin_s, out_s, wqkv_s, wphi_s, wo_s, wop_s, win_s, wsp_s, bsp_s, gb_s, gbo_s, wout_s,
    wbig_s, xn_s, rstd_s, p_s, o_s, kvt_s, z_s, kvacc, zacc, dkvt_s, h_s, z2n_s, g_s,
    dwbig, dwo, dwin, dwout, gwphi_s, sems,
):
    def cp(src, dst, k):
        return pltpu.make_async_copy(src, dst, sems.at[k])

    c_x = cp(x_hbm, xin_s, 0)
    c_wqkv = cp(wqkv_hbm, wqkv_s, 1)
    c_wphi = cp(wphi_hbm, wphi_s, 2)
    c_wo = cp(wo_hbm, wo_s, 3)
    c_win = cp(win_hbm, win_s, 4)
    c_wsp = cp(wsp_hbm, wsp_s, 5)
    c_bsp = cp(bsp_hbm, bsp_s, 6)
    c_wout = cp(wout_hbm, wout_s, 7)
    c_gout = cp(gout_hbm, out_s, 8)
    for c in (c_wqkv, c_wphi, c_wo, c_x):
        c.start()

    def loop(body, name):
        rr = RR.get(name, R)
        with jax.named_scope(name):
            jax.lax.fori_loop(0, S // rr, lambda i, c: (body(_rows(i, rr)), c)[1], 0)

    def iota(shape, dim):
        return jax.lax.broadcasted_iota(jnp.int32, shape, dim)

    def lane_decode(c):
        g1 = c >= 320
        cc = jnp.where(g1, c - 320, c)
        slot = cc >> 4
        e = jnp.where(g1, jnp.where(slot < 4, slot + 16, slot - 4), slot)
        head = (cc & 15) + jnp.where(g1, 16, 0)
        return head, e

    def perm_mat():
        head, e = lane_decode(iota((D, D), 1))
        return jnp.where(iota((D, D), 0) == DH * head + e, 1.0, 0.0).astype(BF16)

    def perm_mat_t():
        head, e = lane_decode(iota((D, D), 0))
        return jnp.where(iota((D, D), 1) == DH * head + e, 1.0, 0.0).astype(BF16)

    def expand_mat():
        _, e = lane_decode(iota((128, D), 1))
        return jnp.where(iota((128, D), 0) == e, 1.0, 0.0).astype(BF16)

    def head_mask():
        head, _ = lane_decode(iota((D, D), 1))
        r = iota((D, D), 0)
        lo = DH * head
        return jnp.logical_and(r >= lo, r < lo + DH)

    def wphi_big():
        rep = _nn(wphi_s[...], expand_mat())
        return jnp.where(head_mask(), rep, 0.0).astype(BF16)

    def kv_masked():
        r = iota((384, D), 0)
        c = iota((384, D), 1)
        same = (r & 15) == (c & 15)
        m0 = jnp.logical_and(same, r < 320)
        m1 = jnp.logical_and(same, r >= 64)
        return (jnp.where(m0, kvacc[0], 0.0).astype(BF16), jnp.where(m1, kvacc[1], 0.0).astype(BF16))

    dwbig[...] = jnp.zeros_like(dwbig)
    dwo[...] = jnp.zeros_like(dwo)
    dwin[...] = jnp.zeros_like(dwin)
    dwout[...] = jnp.zeros_like(dwout)
    gb_s[...] = jnp.zeros_like(gb_s)
    pm = perm_mat()
    pmt = perm_mat_t()
    c_wqkv.wait()
    c_wphi.wait()
    c_wo.wait()
    for c in (c_win, c_wsp, c_bsp, c_wout, c_gout):
        c.start()
    wpb = wphi_big()
    wbig_s[:, 0:D] = _bd_nn(wqkv_s[:, 0:D], wpb).astype(BF16)
    wbig_s[:, D:2 * D] = _bd_nn(wqkv_s[:, D:2 * D], wpb).astype(BF16)
    wbig_s[:, 2 * D:3 * D] = _bd_nn(wqkv_s[:, 2 * D:3 * D], pm).astype(BF16)
    wop_s[...] = _bd_left(pmt, wo_s[...]).astype(BF16)

    def zero_kv():
        kvacc[...] = jnp.zeros_like(kvacc)
        zacc[...] = jnp.zeros_like(zacc)

    def pre_ln(layer, r, x):
        xn, rstd = _ln(x)
        xnb = xn.astype(BF16)
        xn_s[layer, r, :] = xnb
        rstd_s[r, layer:layer + 1] = rstd
        return xnb

    def a_fwd1(layer, r, x):
        a = layer // 2
        xnb = pre_ln(layer, r, x)
        pb = _nn(xnb, wbig_s[...]).astype(BF16)
        p_s[a, r, :] = pb
        phik = _cat(_feat(pb[:, D:2 * D].astype(F32)))
        phikb = phik.astype(BF16)
        kvacc[0] += _tn(pb[:, 2 * D:2 * D + 384], phikb[:, 0:D])
        kvacc[1] += _tn(pb[:, 2 * D + 256:3 * D], phikb[:, D:2 * D])
        zacc[...] += jnp.sum(phik, axis=0, keepdims=True)

    def a_fwd_post(layer):
        a = layer // 2
        k0, k1 = kv_masked()
        kvt_s[a, 0] = k0
        kvt_s[a, 1] = k1
        z_s[a] = zacc[...]

    def a_fwd2(layer, r, x):
        a = layer // 2
        phiq = _feat(p_s[a, r, 0:D].astype(F32))
        lo = _lo(phiq[0].shape)
        z = _slabs(z_s[a], 10)
        pqb = _cat(phiq).astype(BF16)
        n0 = _slabs(_nt(pqb[:, 0:D], kvt_s[a, 0]), 3)
        n1 = _slabs(_nt(pqb[:, D:2 * D], kvt_s[a, 1]), 3)
        num = [n0[0], n0[1], n0[2] + n1[0], n1[1], n1[2]]
        den0, den1 = _phi_head_sum([pq * zz for pq, zz in zip(phiq, z)])
        inv = _head_bcast(1.0 / (den0 + 1e-6), 1.0 / (den1 + 1e-6), lo)
        ob = _cat([t * i for t, i in zip(num, inv)]).astype(BF16)
        o_s[a, r, :] = ob
        return x + _nn(ob, wop_s[...])

    def b_fwd1(layer, r, x):
        b = layer // 2
        xnb = pre_ln(layer, r, x)
        hb = _nn(xnb, win_s[...]).astype(BF16)
        h_s[b, r, :] = hb
        z2, _ = _gelu(hb[:, FH:].astype(F32))
        z2n, _ = _ln(z2)
        z2n_s[b, r, :] = z2n.astype(BF16)

    def b_fwd2(layer, r, x, keep_g=True):
        b = layer // 2
        g = _nn(wsp_s[r, :], z2n_s[b]) + bsp_s[r, :].astype(F32)
        gb = g.astype(BF16)
        if keep_g:
            g_s[b, r, :] = gb
        g = gb.astype(F32)
        h1 = h_s[b, r, 0:FH].astype(F32)
        z1, t1 = _gelu(h1)
        u = (z1 * g).astype(BF16)
        return x + _nn(u, wout_s[...]), (h1, z1, t1, g, u)

    def b_bwd1(layer, r, dy, res=None):
        b = layer // 2
        dyb = dy.astype(BF16)
        du = _nt(dyb, wout_s[...])
        if res is None:
            h1 = h_s[b, r, 0:FH].astype(F32)
            z1, t1 = _gelu(h1)
            g = g_s[b, r, :].astype(F32)
            u = (z1 * g).astype(BF16)
        else:
            h1, z1, t1, g, u = res
        dwout[...] += _tn(u, dyb)
        dg = du * z1
        g_s[b, r, :] = dg.astype(BF16)
        gb_s[r, :] += jnp.sum(dg, axis=-1, keepdims=True)
        h_s[b, r, 0:FH] = (du * g * _gelu_grad(h1, t1)).astype(BF16)

    def b_bwd2(layer, r, dy):
        b = layer // 2
        dz2n = _tn(wsp_s[:, r], g_s[b])
        h2 = h_s[b, r, FH:].astype(F32)
        z2, t2 = _gelu(h2)
        z2n, rstd2 = _ln(z2)
        dz2 = _ln_bwd(dz2n, z2n, rstd2)
        dh2 = (dz2 * _gelu_grad(h2, t2)).astype(BF16)
        dh = _cat([h_s[b, r, 0:FH], dh2])
        dxn = _nt(dh, win_s[...])
        xnb = xn_s[layer, r, :]
        dwin[...] += _tn(xnb, dh)
        return dy + _ln_bwd(dxn, xnb.astype(F32), rstd_s[r, layer:layer + 1])

    def a_bwd1(layer, r, dy):
        a = layer // 2
        dyb = dy.astype(BF16)
        do = _slabs(_nt(dyb, wop_s[...]), 5)
        ob = o_s[a, r, :]
        dwo[...] += _tn(ob, dyb)
        o = _slabs(ob.astype(F32), 5)
        phiq = _feat(p_s[a, r, 0:D].astype(F32))
        lo = _lo(phiq[0].shape)
        z = _slabs(z_s[a], 10)
        den0, den1 = _phi_head_sum([pq * zz for pq, zz in zip(phiq, z)])
        i0 = 1.0 / (den0 + 1e-6)
        i1 = 1.0 / (den1 + 1e-6)
        inv = _head_bcast(i0, i1, lo)
        dnum = _cat([t * i for t, i in zip(do, inv)]).astype(BF16)
        q0, q1 = _head_reduce([u * w for u, w in zip(do, o)], lo, jnp.add, 0.0)
        dd0 = -q0 * i0
        dd1 = -q1 * i1
        dden = [dd0] * 5 + [dd1] * 5
        dphiq = _slabs(_nn(dnum[:, 0:384], kvt_s[a, 0]), 5) + _slabs(_nn(dnum[:, 256:D], kvt_s[a, 1]), 5)
        dphiq = [t + dd * zz for t, dd, zz in zip(dphiq, dden, z)]
        pqb = _cat(phiq).astype(BF16)
        kvacc[0] += _tn(dnum[:, 0:384], pqb[:, 0:D])
        kvacc[1] += _tn(dnum[:, 256:D], pqb[:, D:2 * D])
        zacc[...] += jnp.sum(_cat([pq * dd for pq, dd in zip(phiq, dden)]), axis=0, keepdims=True)
        p_s[a, r, 0:D] = _cat(_feat_bwd(phiq, dphiq)).astype(BF16)

    def a_bwd_post():
        k0, k1 = kv_masked()
        dkvt_s[0] = k0
        dkvt_s[1] = k1

    def a_bwd2a(layer, r):
        a = layer // 2
        phik = _feat(p_s[a, r, D:2 * D].astype(F32))
        vb = p_s[a, r, 2 * D:3 * D]
        dz = _slabs(zacc[...], 10)
        dphik = _slabs(_nn(vb[:, 0:384], dkvt_s[0]), 5) + _slabs(_nn(vb[:, 256:D], dkvt_s[1]), 5)
        dphik = [t + zz for t, zz in zip(dphik, dz)]
        pkb = _cat(phik).astype(BF16)
        n0 = _slabs(_nt(pkb[:, 0:D], dkvt_s[0]), 3)
        n1 = _slabs(_nt(pkb[:, D:2 * D], dkvt_s[1]), 3)
        dv = [n0[0], n0[1], n0[2] + n1[0], n1[1], n1[2]]
        p_s[a, r, D:3 * D] = _cat(_feat_bwd(phik, dphik) + dv).astype(BF16)

    def a_bwd2b(layer, r, dy):
        a = layer // 2
        dp = p_s[a, r, :]
        dxn = _nt(dp, wbig_s[...])
        xnb = xn_s[layer, r, :]
        dwbig[...] += _tn(xnb, dp)
        return dy + _ln_bwd(dxn, xnb.astype(F32), rstd_s[r, layer:layer + 1])

    def skew(stage_a, stage_b, name):
        rr = RR.get(name, R)
        nch = S // rr
        with jax.named_scope(name):
            stage_a(_rows(0, rr))

            def body(i, c):
                stage_b(_rows(i - 1, rr))
                stage_a(_rows(i, rr))
                return c

            jax.lax.fori_loop(1, nch, body, 0)
            stage_b(_rows(nch - 1, rr))

    c_x.wait()
    zero_kv()

    def f1(r):
        x = xin_s[r, :].astype(F32)
        x_s[r, :] = x
        a_fwd1(0, r, x)

    loop(f1, 'F1')
    a_fwd_post(0)
    c_win.wait()

    def f2a(r):
        x_s[r, :] = a_fwd2(0, r, x_s[r, :])

    skew(f2a, lambda r: b_fwd1(1, r, x_s[r, :]), 'F2')
    c_wsp.wait()
    c_bsp.wait()
    c_wout.wait()
    zero_kv()

    def f3a(r):
        x, _ = b_fwd2(1, r, x_s[r, :])
        x_s[r, :] = x

    def f3b(r):
        a_fwd1(2, r, x_s[r, :])

    skew(f3a, f3b, 'F3')
    a_fwd_post(2)

    def f4a(r):
        x_s[r, :] = a_fwd2(2, r, x_s[r, :])

    skew(f4a, lambda r: b_fwd1(3, r, x_s[r, :]), 'F4')
    c_gout.wait()

    def f5(r):
        x, res = b_fwd2(3, r, x_s[r, :], keep_g=False)
        xin_s[r, :] = x.astype(BF16)
        dy = out_s[r, :].astype(F32)
        x_s[r, :] = dy
        b_bwd1(3, r, dy, res)

    loop(f5, 'F5')
    c_out = cp(xin_s, out_hbm, 9)
    c_out.start()

    zero_kv()

    def g1a(r):
        x_s[r, :] = b_bwd2(3, r, x_s[r, :])

    skew(g1a, lambda r: a_bwd1(2, r, x_s[r, :]), 'G1')
    a_bwd_post()

    def g2a(r):
        a_bwd2a(2, r)
        x_s[r, :] = a_bwd2b(2, r, x_s[r, :])

    skew(g2a, lambda r: b_bwd1(1, r, x_s[r, :]), 'G2')
    zero_kv()

    def g3a(r):
        x_s[r, :] = b_bwd2(1, r, x_s[r, :])

    skew(g3a, lambda r: a_bwd1(0, r, x_s[r, :]), 'G3')
    a_bwd_post()

    win_s[...] = dwin[...].astype(BF16)
    wout_s[...] = dwout[...].astype(BF16)
    gbo_s[...] = gb_s[...].astype(BF16)
    c_gwin = cp(win_s, gwin_hbm, 11)
    c_gwout = cp(wout_s, gwout_hbm, 12)
    c_gb = cp(gbo_s, gbsp_hbm, 13)
    for c in (c_gwin, c_gwout, c_gb):
        c.start()

    def g4b(r):
        out_s[r, :] = a_bwd2b(0, r, x_s[r, :]).astype(BF16)

    skew(lambda r: a_bwd2a(0, r), g4b, 'G4')
    c_gx = cp(out_s, gx_hbm, 14)
    c_gx.start()

    dq = dwbig[:, 0:D].astype(BF16)
    dk = dwbig[:, D:2 * D].astype(BF16)
    dvv = dwbig[:, 2 * D:3 * D].astype(BF16)
    wpb = wphi_big()
    hm = head_mask()
    ex = expand_mat()
    m0 = _tn(wqkv_s[:, 0:384], dq[:, 0:384]) + _tn(wqkv_s[:, D:D + 384], dk[:, 0:384])
    m1 = (_tn(wqkv_s[:, 256:D], dq[:, 256:D]) + _tn(wqkv_s[:, D + 256:2 * D], dk[:, 256:D]))
    r384 = iota((384, 384), 0)
    m0 = jnp.where(jnp.logical_and(hm[0:384, 0:384], r384 < 320), m0, 0.0).astype(BF16)
    m1 = jnp.where(jnp.logical_and(hm[256:D, 256:D], r384 >= 64), m1, 0.0).astype(BF16)
    w0 = _nt(m0, ex[:, 0:384])
    w1 = _nt(m1, ex[:, 256:D])
    gwphi_s[0:256, :] = w0[0:256].astype(BF16)
    gwphi_s[256:384, :] = (w0[256:384] + w1[0:128]).astype(BF16)
    gwphi_s[384:D, :] = w1[128:384].astype(BF16)
    c_gwphi = cp(gwphi_s, gwphi_hbm, 15)
    c_gwphi.start()
    pm = perm_mat()
    wbig_s[:, 0:D] = _bd_nt(dq, wpb).astype(BF16)
    wbig_s[:, D:2 * D] = _bd_nt(dk, wpb).astype(BF16)
    wbig_s[:, 2 * D:3 * D] = _bd_nt(dvv, pm).astype(BF16)
    c_gwqkv = cp(wbig_s, gwqkv_hbm, 16)
    c_gwqkv.start()
    wo_s[...] = _bd_left(pm, dwo[...].astype(BF16)).astype(BF16)
    c_gwo = cp(wo_s, gwo_hbm, 17)
    c_gwo.start()

    def wsp_loop(r):
        wsp_s[r, :] = (_nt(g_s[0, r, :], z2n_s[0]) + _nt(g_s[1, r, :], z2n_s[1])).astype(BF16)
        pltpu.make_async_copy(wsp_s.at[r], gwsp_hbm.at[r], sems.at[10]).start()

    loop(wsp_loop, 'wsp')

    for c in (c_out, c_gwin, c_gwout, c_gb, c_gx, c_gwphi, c_gwqkv, c_gwo):
        c.wait()
    cp(wsp_s, gwsp_hbm, 10).wait()


@jax.jit
def pallas_interleave_layers__linear_kernel_hedgehog__mixer_gmlp__prompt_kernel(
    A_x: jax.Array,
    A_wqkv: jax.Array,
    A_w_phi: jax.Array,
    A_wo: jax.Array,
    B_x: jax.Array,
    B_w_in: jax.Array,
    B_w_sp: jax.Array,
    B_b_sp: jax.Array,
    B_w_out: jax.Array,
    grad_out: jax.Array,
):
    del B_x
    x = A_x.reshape(S, D)
    gout = grad_out.reshape(S, D)
    wphi = jnp.pad(A_w_phi.reshape(D, DH), ((0, 0), (0, 128 - DH)))
    bsp = B_b_sp.reshape(S, 1)

    any_spec = pl.BlockSpec(memory_space=pl.ANY)
    out_shape = (
        jax.ShapeDtypeStruct((S, D), BF16),
        jax.ShapeDtypeStruct((S, D), BF16),
        jax.ShapeDtypeStruct((D, 3 * D), BF16),
        jax.ShapeDtypeStruct((D, 128), BF16),
        jax.ShapeDtypeStruct((D, D), BF16),
        jax.ShapeDtypeStruct((D, FF), BF16),
        jax.ShapeDtypeStruct((S, S), BF16),
        jax.ShapeDtypeStruct((S, 1), BF16),
        jax.ShapeDtypeStruct((FH, D), BF16),
    )
    scratch = [
        pltpu.VMEM((S, D), F32),
        pltpu.VMEM((S, D), BF16),
        pltpu.VMEM((S, D), BF16),
        pltpu.VMEM((D, 3 * D), BF16),
        pltpu.VMEM((D, 128), BF16),
        pltpu.VMEM((D, D), BF16),
        pltpu.VMEM((D, D), BF16),
        pltpu.VMEM((D, FF), BF16),
        pltpu.VMEM((S, S), BF16),
        pltpu.VMEM((S, 1), BF16),
        pltpu.VMEM((S, 1), F32),
        pltpu.VMEM((S, 1), BF16),
        pltpu.VMEM((FH, D), BF16),
        pltpu.VMEM((D, 3 * D), BF16),
        pltpu.VMEM((4, S, D), BF16),
        pltpu.VMEM((S, 128), F32),
        pltpu.VMEM((2, S, 3 * D), BF16),
        pltpu.VMEM((2, S, D), BF16),
        pltpu.VMEM((2, 2, 384, D), BF16),
        pltpu.VMEM((2, 1, F2), F32),
        pltpu.VMEM((2, 384, D), F32),
        pltpu.VMEM((1, F2), F32),
        pltpu.VMEM((2, 384, D), BF16),
        pltpu.VMEM((2, S, FF), BF16),
        pltpu.VMEM((2, S, FH), BF16),
        pltpu.VMEM((2, S, FH), BF16),
        pltpu.VMEM((D, 3 * D), F32),
        pltpu.VMEM((D, D), F32),
        pltpu.VMEM((D, FF), F32),
        pltpu.VMEM((FH, D), F32),
        pltpu.VMEM((D, 128), BF16),
        pltpu.SemaphoreType.DMA((18,)),
    ]
    outs = pl.pallas_call(
        _kernel,
        out_shape=out_shape,
        in_specs=[any_spec] * 9,
        out_specs=tuple([any_spec] * 9),
        scratch_shapes=scratch,
        compiler_params=pltpu.CompilerParams(vmem_limit_bytes=127 * 1024 * 1024),
    )(x, A_wqkv, wphi, A_wo, B_w_in, B_w_sp, bsp, B_w_out, gout)
    out, gx, gwqkv, gwphi, gwo, gwin, gwsp, gbsp, gwout = outs
    return (
        out.reshape(1, S, D),
        gx.reshape(1, S, D),
        gwqkv,
        gwphi[:, :DH].reshape(H, DH, DH),
        gwo,
        gwin,
        gwsp,
        gbsp.reshape(S),
        gwout,
    )
```

```python
import jax
import jax.numpy as jnp
import jax.experimental.pallas as pl
import jax.experimental.pallas.tpu as pltpu

F32 = jnp.float32
BF16 = jnp.bfloat16

S = 2048
D = 640
H = 32
DH = 20
F2 = 2 * DH * H
FF = 1536
FH = 768
EPS = 1e-5
R = 256
NCH = S // R
RR = {}

_C0 = 0.7978845608028654
_C1 = 0.044715


def _nn(a, b):
    return jnp.dot(a, b, preferred_element_type=F32)


def _nt(a, b):
    return jax.lax.dot_general(a, b, (((1,), (1,)), ((), ())), preferred_element_type=F32)


def _tn(a, b):
    return jax.lax.dot_general(a, b, (((0,), (0,)), ((), ())), preferred_element_type=F32)


def _ln(x):
    m = jnp.mean(x, axis=-1, keepdims=True)
    xc = x - m
    v = jnp.mean(xc * xc, axis=-1, keepdims=True)
    rstd = jax.lax.rsqrt(v + EPS)
    return xc * rstd, rstd


def _ln_bwd(dxn, xn, rstd):
    a = jnp.mean(dxn, axis=-1, keepdims=True)
    b = jnp.mean(dxn * xn, axis=-1, keepdims=True)
    return rstd * (dxn - a - xn * b)


def _gelu(x):
    t = jnp.tanh(_C0 * (x + _C1 * x * x * x))
    return 0.5 * x * (1.0 + t), t


def _gelu_grad(x, t):
    return 0.5 * (1.0 + t) + 0.5 * x * (1.0 - t * t) * _C0 * (1.0 + 3.0 * _C1 * x * x)


def _grp(a, op):
    a = op(a, pltpu.roll(a, 64, 1))
    a = op(a, pltpu.roll(a, 32, 1))
    a = op(a, pltpu.roll(a, 16, 1))
    return a


def _slabs(a, n):
    return [a[:, j * 128:(j + 1) * 128] for j in range(n)]


def _cat(xs):
    return jnp.concatenate(xs, axis=1)


def _lo(shape):
    return jax.lax.broadcasted_iota(jnp.int32, shape, 1) < 64


def _head_reduce(t, lo, op, fill):
    a0 = op(op(t[0], t[1]), jnp.where(lo, t[2], fill))
    a1 = op(op(t[3], t[4]), jnp.where(lo, fill, t[2]))
    return _grp(a0, op), _grp(a1, op)


def _head_bcast(r0, r1, lo):
    rx = jnp.where(lo, r0, r1)
    return [r0, r0, rx, r1, r1]


def _feat(p):
    t = _slabs(p, 5)
    lo = _lo(t[0].shape)
    mx = _head_bcast(*_head_reduce(t, lo, jnp.maximum, -jnp.inf), lo)
    mn = _head_bcast(*_head_reduce(t, lo, jnp.minimum, jnp.inf), lo)
    ep = [jnp.exp(a - m) for a, m in zip(t, mx)]
    en = [jnp.exp(m - a) for a, m in zip(t, mn)]
    sp0, sp1 = _head_reduce(ep, lo, jnp.add, 0.0)
    sn0, sn1 = _head_reduce(en, lo, jnp.add, 0.0)
    ip = _head_bcast(1.0 / sp0, 1.0 / sp1, lo)
    inn = _head_bcast(1.0 / sn0, 1.0 / sn1, lo)
    fp = [e * i for e, i in zip(ep, ip)]
    fn = [e * i for e, i in zip(en, inn)]
    fnx = pltpu.roll(fn[2], 64, 1)
    px0 = jnp.where(lo, fp[2], fnx)
    px1 = jnp.where(lo, fnx, fp[2])
    return [fp[0], fp[1], fn[0], fn[1], px0, px1, fp[3], fp[4], fn[3], fn[4]]


def _phi_head_sum(t):
    s0 = (t[0] + t[1]) + (t[2] + t[3]) + t[4]
    s1 = (t[6] + t[7]) + (t[8] + t[9]) + t[5]
    return _grp(s0, jnp.add), _grp(s1, jnp.add)


def _feat_bwd(phi, dphi):
    lo = _lo(phi[0].shape)
    t = [a * b for a, b in zip(phi, dphi)]
    sp0 = _grp(t[0] + t[1] + jnp.where(lo, t[4], 0.0), jnp.add)
    sn0 = _grp(t[2] + t[3] + jnp.where(lo, 0.0, t[4]), jnp.add)
    sp1 = _grp(t[6] + t[7] + jnp.where(lo, 0.0, t[5]), jnp.add)
    sn1 = _grp(t[8] + t[9] + jnp.where(lo, t[5], 0.0), jnp.add)
    d0 = (t[0] - phi[0] * sp0) - (t[2] - phi[2] * sn0)
    d1 = (t[1] - phi[1] * sp0) - (t[3] - phi[3] * sn0)
    d3 = (t[6] - phi[6] * sp1) - (t[8] - phi[8] * sn1)
    d4 = (t[7] - phi[7] * sp1) - (t[9] - phi[9] * sn1)
    a0 = t[4] - phi[4] * jnp.where(lo, sp0, sn0)
    a1 = t[5] - phi[5] * jnp.where(lo, sn1, sp1)
    dx = jnp.where(lo, a0, a1) - pltpu.roll(jnp.where(lo, a1, a0), 64, 1)
    return [d0, d1, dx, d3, d4]


def _bd_nn(a, w):
    return _cat([_nn(a[:, 0:384], w[0:384, 0:256]), _nn(a, w[:, 256:384]), _nn(a[:, 256:D], w[256:D, 384:D])])


def _bd_nt(a, w):
    return _cat([_nt(a[:, 0:384], w[0:256, 0:384]), _nt(a, w[256:384, :]), _nt(a[:, 256:D], w[384:D, 256:D])])


def _bd_left(w, b):
    return jnp.concatenate(
        [_nn(w[0:256, 0:384], b[0:384]), _nn(w[256:384, :], b), _nn(w[384:D, 256:D], b[256:D])], axis=0)


def _rows(i, rr):
    return pl.ds(pl.multiple_of(i * rr, rr), rr)


def _kernel(
    x_hbm, wqkv_hbm, wphi_hbm, wo_hbm, win_hbm, wsp_hbm, bsp_hbm, wout_hbm, gout_hbm,
    out_hbm, gx_hbm, gwqkv_hbm, gwphi_hbm, gwo_hbm, gwin_hbm, gwsp_hbm, gbsp_hbm, gwout_hbm,
    x_s, xin_s, out_s, wqkv_s, wphi_s, wo_s, wop_s, win_s, wsp_s, bsp_s, gb_s, gbo_s, wout_s,
    wbig_s, xn_s, rstd_s, p_s, o_s, kvt_s, z_s, kvacc, zacc, dkvt_s, h_s, z2n_s, g_s,
    dwbig, dwo, dwin, dwout, gwphi_s, sems,
):
    def cp(src, dst, k):
        return pltpu.make_async_copy(src, dst, sems.at[k])

    c_x = cp(x_hbm, xin_s, 0)
    c_wqkv = cp(wqkv_hbm, wqkv_s, 1)
    c_wphi = cp(wphi_hbm, wphi_s, 2)
    c_wo = cp(wo_hbm, wo_s, 3)
    c_win = cp(win_hbm, win_s, 4)
    c_wsp = cp(wsp_hbm, wsp_s, 5)
    c_bsp = cp(bsp_hbm, bsp_s, 6)
    c_wout = cp(wout_hbm, wout_s, 7)
    c_gout = cp(gout_hbm, out_s, 8)
    for c in (c_wqkv, c_wphi, c_wo, c_x):
        c.start()

    def loop(body, name):
        rr = RR.get(name, R)
        with jax.named_scope(name):
            jax.lax.fori_loop(0, S // rr, lambda i, c: (body(_rows(i, rr)), c)[1], 0)

    def iota(shape, dim):
        return jax.lax.broadcasted_iota(jnp.int32, shape, dim)

    def lane_decode(c):
        g1 = c >= 320
        cc = jnp.where(g1, c - 320, c)
        slot = cc >> 4
        e = jnp.where(g1, jnp.where(slot < 4, slot + 16, slot - 4), slot)
        head = (cc & 15) + jnp.where(g1, 16, 0)
        return head, e

    def perm_mat():
        head, e = lane_decode(iota((D, D), 1))
        return jnp.where(iota((D, D), 0) == DH * head + e, 1.0, 0.0).astype(BF16)

    def perm_mat_t():
        head, e = lane_decode(iota((D, D), 0))
        return jnp.where(iota((D, D), 1) == DH * head + e, 1.0, 0.0).astype(BF16)

    def expand_mat():
        _, e = lane_decode(iota((128, D), 1))
        return jnp.where(iota((128, D), 0) == e, 1.0, 0.0).astype(BF16)

    def head_mask():
        head, _ = lane_decode(iota((D, D), 1))
        r = iota((D, D), 0)
        lo = DH * head
        return jnp.logical_and(r >= lo, r < lo + DH)

    def wphi_big():
        rep = _nn(wphi_s[...], expand_mat())
        return jnp.where(head_mask(), rep, 0.0).astype(BF16)

    def kv_masked():
        r = iota((384, D), 0)
        c = iota((384, D), 1)
        same = (r & 15) == (c & 15)
        m0 = jnp.logical_and(same, r < 320)
        m1 = jnp.logical_and(same, r >= 64)
        return (jnp.where(m0, kvacc[0], 0.0).astype(BF16), jnp.where(m1, kvacc[1], 0.0).astype(BF16))

    dwbig[...] = jnp.zeros_like(dwbig)
    dwo[...] = jnp.zeros_like(dwo)
    dwin[...] = jnp.zeros_like(dwin)
    dwout[...] = jnp.zeros_like(dwout)
    gb_s[...] = jnp.zeros_like(gb_s)
    pm = perm_mat()
    pmt = perm_mat_t()
    c_wqkv.wait()
    c_wphi.wait()
    c_wo.wait()
    for c in (c_win, c_wsp, c_bsp, c_wout, c_gout):
        c.start()
    wpb = wphi_big()
    wbig_s[:, 0:D] = _bd_nn(wqkv_s[:, 0:D], wpb).astype(BF16)
    wbig_s[:, D:2 * D] = _bd_nn(wqkv_s[:, D:2 * D], wpb).astype(BF16)
    wbig_s[:, 2 * D:3 * D] = _bd_nn(wqkv_s[:, 2 * D:3 * D], pm).astype(BF16)
    wop_s[...] = _bd_left(pmt, wo_s[...]).astype(BF16)

    def zero_kv():
        kvacc[...] = jnp.zeros_like(kvacc)
        zacc[...] = jnp.zeros_like(zacc)

    def pre_ln(layer, r, x):
        xn, rstd = _ln(x)
        xnb = xn.astype(BF16)
        xn_s[layer, r, :] = xnb
        rstd_s[r, layer:layer + 1] = rstd
        return xnb

    def a_fwd1(layer, r, x):
        a = layer // 2
        xnb = pre_ln(layer, r, x)
        pb = _nn(xnb, wbig_s[...]).astype(BF16)
        p_s[a, r, :] = pb
        phik = _cat(_feat(pb[:, D:2 * D].astype(F32)))
        phikb = phik.astype(BF16)
        kvacc[0] += _tn(pb[:, 2 * D:2 * D + 384], phikb[:, 0:D])
        kvacc[1] += _tn(pb[:, 2 * D + 256:3 * D], phikb[:, D:2 * D])
        zacc[...] += jnp.sum(phik, axis=0, keepdims=True)

    def a_fwd_post(layer):
        a = layer // 2
        k0, k1 = kv_masked()
        kvt_s[a, 0] = k0
        kvt_s[a, 1] = k1
        z_s[a] = zacc[...]

    def a_fwd2(layer, r, x):
        a = layer // 2
        phiq = _feat(p_s[a, r, 0:D].astype(F32))
        lo = _lo(phiq[0].shape)
        z = _slabs(z_s[a], 10)
        pqb = _cat(phiq).astype(BF16)
        n0 = _slabs(_nt(pqb[:, 0:D], kvt_s[a, 0]), 3)
        n1 = _slabs(_nt(pqb[:, D:2 * D], kvt_s[a, 1]), 3)
        num = [n0[0], n0[1], n0[2] + n1[0], n1[1], n1[2]]
        den0, den1 = _phi_head_sum([pq * zz for pq, zz in zip(phiq, z)])
        inv = _head_bcast(1.0 / (den0 + 1e-6), 1.0 / (den1 + 1e-6), lo)
        ob = _cat([t * i for t, i in zip(num, inv)]).astype(BF16)
        o_s[a, r, :] = ob
        return x + _nn(ob, wop_s[...])

    def b_fwd1(layer, r, x):
        b = layer // 2
        xnb = pre_ln(layer, r, x)
        hb = _nn(xnb, win_s[...]).astype(BF16)
        h_s[b, r, :] = hb
        z2, _ = _gelu(hb[:, FH:].astype(F32))
        z2n, _ = _ln(z2)
        z2n_s[b, r, :] = z2n.astype(BF16)

    def b_fwd2(layer, r, x, keep_g=True):
        b = layer // 2
        g = _nn(wsp_s[r, :], z2n_s[b]) + bsp_s[r, :].astype(F32)
        gb = g.astype(BF16)
        if keep_g:
            g_s[b, r, :] = gb
        g = gb.astype(F32)
        h1 = h_s[b, r, 0:FH].astype(F32)
        z1, t1 = _gelu(h1)
        u = (z1 * g).astype(BF16)
        return x + _nn(u, wout_s[...]), (h1, z1, t1, g, u)

    def b_bwd1(layer, r, dy, res=None):
        b = layer // 2
        dyb = dy.astype(BF16)
        du = _nt(dyb, wout_s[...])
        if res is None:
            h1 = h_s[b, r, 0:FH].astype(F32)
            z1, t1 = _gelu(h1)
            g = g_s[b, r, :].astype(F32)
            u = (z1 * g).astype(BF16)
        else:
            h1, z1, t1, g, u = res
        dwout[...] += _tn(u, dyb)
        dg = du * z1
        g_s[b, r, :] = dg.astype(BF16)
        gb_s[r, :] += jnp.sum(dg, axis=-1, keepdims=True)
        h_s[b, r, 0:FH] = (du * g * _gelu_grad(h1, t1)).astype(BF16)

    def b_bwd2(layer, r, dy):
        b = layer // 2
        dz2n = _tn(wsp_s[:, r], g_s[b])
        h2 = h_s[b, r, FH:].astype(F32)
        z2, t2 = _gelu(h2)
        z2n, rstd2 = _ln(z2)
        dz2 = _ln_bwd(dz2n, z2n, rstd2)
        dh2 = (dz2 * _gelu_grad(h2, t2)).astype(BF16)
        dh = _cat([h_s[b, r, 0:FH], dh2])
        dxn = _nt(dh, win_s[...])
        xnb = xn_s[layer, r, :]
        dwin[...] += _tn(xnb, dh)
        return dy + _ln_bwd(dxn, xnb.astype(F32), rstd_s[r, layer:layer + 1])

    def a_bwd1(layer, r, dy):
        a = layer // 2
        dyb = dy.astype(BF16)
        do = _slabs(_nt(dyb, wop_s[...]), 5)
        ob = o_s[a, r, :]
        dwo[...] += _tn(ob, dyb)
        o = _slabs(ob.astype(F32), 5)
        phiq = _feat(p_s[a, r, 0:D].astype(F32))
        lo = _lo(phiq[0].shape)
        z = _slabs(z_s[a], 10)
        den0, den1 = _phi_head_sum([pq * zz for pq, zz in zip(phiq, z)])
        i0 = 1.0 / (den0 + 1e-6)
        i1 = 1.0 / (den1 + 1e-6)
        inv = _head_bcast(i0, i1, lo)
        dnum = _cat([t * i for t, i in zip(do, inv)]).astype(BF16)
        q0, q1 = _head_reduce([u * w for u, w in zip(do, o)], lo, jnp.add, 0.0)
        dd0 = -q0 * i0
        dd1 = -q1 * i1
        dden = [dd0] * 5 + [dd1] * 5
        dphiq = _slabs(_nn(dnum[:, 0:384], kvt_s[a, 0]), 5) + _slabs(_nn(dnum[:, 256:D], kvt_s[a, 1]), 5)
        dphiq = [t + dd * zz for t, dd, zz in zip(dphiq, dden, z)]
        pqb = _cat(phiq).astype(BF16)
        kvacc[0] += _tn(dnum[:, 0:384], pqb[:, 0:D])
        kvacc[1] += _tn(dnum[:, 256:D], pqb[:, D:2 * D])
        zacc[...] += jnp.sum(_cat([pq * dd for pq, dd in zip(phiq, dden)]), axis=0, keepdims=True)
        p_s[a, r, 0:D] = _cat(_feat_bwd(phiq, dphiq)).astype(BF16)

    def a_bwd_post():
        k0, k1 = kv_masked()
        dkvt_s[0] = k0
        dkvt_s[1] = k1

    def a_bwd2a(layer, r):
        a = layer // 2
        phik = _feat(p_s[a, r, D:2 * D].astype(F32))
        vb = p_s[a, r, 2 * D:3 * D]
        dz = _slabs(zacc[...], 10)
        dphik = _slabs(_nn(vb[:, 0:384], dkvt_s[0]), 5) + _slabs(_nn(vb[:, 256:D], dkvt_s[1]), 5)
        dphik = [t + zz for t, zz in zip(dphik, dz)]
        pkb = _cat(phik).astype(BF16)
        n0 = _slabs(_nt(pkb[:, 0:D], dkvt_s[0]), 3)
        n1 = _slabs(_nt(pkb[:, D:2 * D], dkvt_s[1]), 3)
        dv = [n0[0], n0[1], n0[2] + n1[0], n1[1], n1[2]]
        p_s[a, r, D:3 * D] = _cat(_feat_bwd(phik, dphik) + dv).astype(BF16)

    def a_bwd2b(layer, r, dy):
        a = layer // 2
        dp = p_s[a, r, :]
        dxn = _nt(dp, wbig_s[...])
        xnb = xn_s[layer, r, :]
        dwbig[...] += _tn(xnb, dp)
        return dy + _ln_bwd(dxn, xnb.astype(F32), rstd_s[r, layer:layer + 1])

    def skew(stage_a, stage_b, name):
        rr = RR.get(name, R)
        nch = S // rr
        with jax.named_scope(name):
            stage_a(_rows(0, rr))

            def body(i, c):
                stage_b(_rows(i - 1, rr))
                stage_a(_rows(i, rr))
                return c

            jax.lax.fori_loop(1, nch, body, 0)
            stage_b(_rows(nch - 1, rr))

    c_x.wait()
    zero_kv()

    def f1(r):
        x = xin_s[r, :].astype(F32)
        x_s[r, :] = x
        a_fwd1(0, r, x)

    loop(f1, 'F1')
    a_fwd_post(0)
    c_win.wait()

    def f2a(r):
        x_s[r, :] = a_fwd2(0, r, x_s[r, :])

    skew(f2a, lambda r: b_fwd1(1, r, x_s[r, :]), 'F2')
    c_wsp.wait()
    c_bsp.wait()
    c_wout.wait()
    zero_kv()

    def f3a(r):
        x, _ = b_fwd2(1, r, x_s[r, :])
        x_s[r, :] = x

    def f3b(r):
        a_fwd1(2, r, x_s[r, :])

    skew(f3a, f3b, 'F3')
    a_fwd_post(2)

    def f4a(r):
        x_s[r, :] = a_fwd2(2, r, x_s[r, :])

    skew(f4a, lambda r: b_fwd1(3, r, x_s[r, :]), 'F4')
    c_gout.wait()

    def f5(r):
        x, res = b_fwd2(3, r, x_s[r, :], keep_g=False)
        xin_s[r, :] = x.astype(BF16)
        dy = out_s[r, :].astype(F32)
        x_s[r, :] = dy
        b_bwd1(3, r, dy, res)

    loop(f5, 'F5')
    c_out = cp(xin_s, out_hbm, 9)
    c_out.start()

    zero_kv()

    def g1(r):
        dy = b_bwd2(3, r, x_s[r, :])
        x_s[r, :] = dy
        a_bwd1(2, r, dy)

    loop(g1, 'G1')
    a_bwd_post()

    def g2a(r):
        a_bwd2a(2, r)
        x_s[r, :] = a_bwd2b(2, r, x_s[r, :])

    skew(g2a, lambda r: b_bwd1(1, r, x_s[r, :]), 'G2')
    zero_kv()

    def g3(r):
        dy = b_bwd2(1, r, x_s[r, :])
        x_s[r, :] = dy
        a_bwd1(0, r, dy)

    loop(g3, 'G3')
    a_bwd_post()

    win_s[...] = dwin[...].astype(BF16)
    wout_s[...] = dwout[...].astype(BF16)
    gbo_s[...] = gb_s[...].astype(BF16)
    c_gwin = cp(win_s, gwin_hbm, 11)
    c_gwout = cp(wout_s, gwout_hbm, 12)
    c_gb = cp(gbo_s, gbsp_hbm, 13)
    for c in (c_gwin, c_gwout, c_gb):
        c.start()

    def g4b(r):
        out_s[r, :] = a_bwd2b(0, r, x_s[r, :]).astype(BF16)

    skew(lambda r: a_bwd2a(0, r), g4b, 'G4')
    c_gx = cp(out_s, gx_hbm, 14)
    c_gx.start()

    dq = dwbig[:, 0:D].astype(BF16)
    dk = dwbig[:, D:2 * D].astype(BF16)
    dvv = dwbig[:, 2 * D:3 * D].astype(BF16)
    wpb = wphi_big()
    hm = head_mask()
    ex = expand_mat()
    m0 = _tn(wqkv_s[:, 0:384], dq[:, 0:384]) + _tn(wqkv_s[:, D:D + 384], dk[:, 0:384])
    m1 = (_tn(wqkv_s[:, 256:D], dq[:, 256:D]) + _tn(wqkv_s[:, D + 256:2 * D], dk[:, 256:D]))
    r384 = iota((384, 384), 0)
    m0 = jnp.where(jnp.logical_and(hm[0:384, 0:384], r384 < 320), m0, 0.0).astype(BF16)
    m1 = jnp.where(jnp.logical_and(hm[256:D, 256:D], r384 >= 64), m1, 0.0).astype(BF16)
    w0 = _nt(m0, ex[:, 0:384])
    w1 = _nt(m1, ex[:, 256:D])
    gwphi_s[0:256, :] = w0[0:256].astype(BF16)
    gwphi_s[256:384, :] = (w0[256:384] + w1[0:128]).astype(BF16)
    gwphi_s[384:D, :] = w1[128:384].astype(BF16)
    c_gwphi = cp(gwphi_s, gwphi_hbm, 15)
    c_gwphi.start()
    pm = perm_mat()
    wbig_s[:, 0:D] = _bd_nt(dq, wpb).astype(BF16)
    wbig_s[:, D:2 * D] = _bd_nt(dk, wpb).astype(BF16)
    wbig_s[:, 2 * D:3 * D] = _bd_nt(dvv, pm).astype(BF16)
    c_gwqkv = cp(wbig_s, gwqkv_hbm, 16)
    c_gwqkv.start()
    wo_s[...] = _bd_left(pm, dwo[...].astype(BF16)).astype(BF16)
    c_gwo = cp(wo_s, gwo_hbm, 17)
    c_gwo.start()

    def wsp_loop(r):
        wsp_s[r, :] = (_nt(g_s[0, r, :], z2n_s[0]) + _nt(g_s[1, r, :], z2n_s[1])).astype(BF16)
        pltpu.make_async_copy(wsp_s.at[r], gwsp_hbm.at[r], sems.at[10]).start()

    loop(wsp_loop, 'wsp')

    for c in (c_out, c_gwin, c_gwout, c_gb, c_gx, c_gwphi, c_gwqkv, c_gwo):
        c.wait()
    cp(wsp_s, gwsp_hbm, 10).wait()


@jax.jit
def pallas_interleave_layers__linear_kernel_hedgehog__mixer_gmlp__prompt_kernel(
    A_x: jax.Array,
    A_wqkv: jax.Array,
    A_w_phi: jax.Array,
    A_wo: jax.Array,
    B_x: jax.Array,
    B_w_in: jax.Array,
    B_w_sp: jax.Array,
    B_b_sp: jax.Array,
    B_w_out: jax.Array,
    grad_out: jax.Array,
):
    del B_x
    x = A_x.reshape(S, D)
    gout = grad_out.reshape(S, D)
    wphi = jnp.pad(A_w_phi.reshape(D, DH), ((0, 0), (0, 128 - DH)))
    bsp = B_b_sp.reshape(S, 1)

    any_spec = pl.BlockSpec(memory_space=pl.ANY)
    out_shape = (
        jax.ShapeDtypeStruct((S, D), BF16),
        jax.ShapeDtypeStruct((S, D), BF16),
        jax.ShapeDtypeStruct((D, 3 * D), BF16),
        jax.ShapeDtypeStruct((D, 128), BF16),
        jax.ShapeDtypeStruct((D, D), BF16),
        jax.ShapeDtypeStruct((D, FF), BF16),
        jax.ShapeDtypeStruct((S, S), BF16),
        jax.ShapeDtypeStruct((S, 1), BF16),
        jax.ShapeDtypeStruct((FH, D), BF16),
    )
    scratch = [
        pltpu.VMEM((S, D), F32),
        pltpu.VMEM((S, D), BF16),
        pltpu.VMEM((S, D), BF16),
        pltpu.VMEM((D, 3 * D), BF16),
        pltpu.VMEM((D, 128), BF16),
        pltpu.VMEM((D, D), BF16),
        pltpu.VMEM((D, D), BF16),
        pltpu.VMEM((D, FF), BF16),
        pltpu.VMEM((S, S), BF16),
        pltpu.VMEM((S, 1), BF16),
        pltpu.VMEM((S, 1), F32),
        pltpu.VMEM((S, 1), BF16),
        pltpu.VMEM((FH, D), BF16),
        pltpu.VMEM((D, 3 * D), BF16),
        pltpu.VMEM((4, S, D), BF16),
        pltpu.VMEM((S, 128), F32),
        pltpu.VMEM((2, S, 3 * D), BF16),
        pltpu.VMEM((2, S, D), BF16),
        pltpu.VMEM((2, 2, 384, D), BF16),
        pltpu.VMEM((2, 1, F2), F32),
        pltpu.VMEM((2, 384, D), F32),
        pltpu.VMEM((1, F2), F32),
        pltpu.VMEM((2, 384, D), BF16),
        pltpu.VMEM((2, S, FF), BF16),
        pltpu.VMEM((2, S, FH), BF16),
        pltpu.VMEM((2, S, FH), BF16),
        pltpu.VMEM((D, 3 * D), F32),
        pltpu.VMEM((D, D), F32),
        pltpu.VMEM((D, FF), F32),
        pltpu.VMEM((FH, D), F32),
        pltpu.VMEM((D, 128), BF16),
        pltpu.SemaphoreType.DMA((18,)),
    ]
    outs = pl.pallas_call(
        _kernel,
        out_shape=out_shape,
        in_specs=[any_spec] * 9,
        out_specs=tuple([any_spec] * 9),
        scratch_shapes=scratch,
        compiler_params=pltpu.CompilerParams(vmem_limit_bytes=127 * 1024 * 1024),
    )(x, A_wqkv, wphi, A_wo, B_w_in, B_w_sp, bsp, B_w_out, gout)
    out, gx, gwqkv, gwphi, gwo, gwin, gwsp, gbsp, gwout = outs
    return (
        out.reshape(1, S, D),
        gx.reshape(1, S, D),
        gwqkv,
        gwphi[:, :DH].reshape(H, DH, DH),
        gwo,
        gwin,
        gwsp,
        gbsp.reshape(S),
        gwout,
    )
```
